```python
import os as _os
_os.environ.setdefault("JAX_PLATFORMS", "cpu")
import jax
import jax.numpy as jnp

def _softmax(x, axis=-1):
    return jax.nn.softmax(x, axis=axis)
def _gelu(x):
    return jax.nn.gelu(x, approximate=True)
def _silu(x):
    return jax.nn.silu(x)
def _sigmoid(x):
    return jax.nn.sigmoid(x)
def _layernorm(x, axis=-1, eps=1e-5):
    m = jnp.mean(x, axis=axis, keepdims=True)
    v = jnp.var(x, axis=axis, keepdims=True)
    return (x - m) / jnp.sqrt(v + eps)
def _scatter_add(tgt, idx, src, axis=0):
    return tgt.at[idx].add(src)
def _segment_sum(src, seg, n):
    return jax.ops.segment_sum(src, seg, n)
class _Rng:
    def __init__(self, key):
        self._k = key
    def _next(self):
        self._k, sub = jax.random.split(self._k)
        return sub
    def normal(self, shape):
        return jax.random.normal(self._next(), shape, dtype=jnp.bfloat16)
    def randint(self, lo, hi, shape):
        return jax.random.randint(self._next(), shape, lo, hi, dtype=jnp.int32)
    def uniform(self, shape, lo=0.0, hi=1.0):
        return jax.random.uniform(self._next(), shape, jnp.bfloat16, lo, hi)
    def permutation(self, n):
        return jax.random.permutation(self._next(), n)


kernel_name = 'standalone__gqa_block_cached__near_ridge'

def setup_inputs():
    _rng = _Rng(jax.random.key(int.from_bytes(__import__("os").urandom(4), "little")))
    _w = (lambda a: (lambda t: t.astype(jnp.bfloat16) if jnp.issubdtype(t.dtype, jnp.floating) else t)(jnp.asarray(a)))
    B, Sq, D = 32, 112, 448
    Hq, Hkv, Sk, Dh = 16, 8, 512, 256
    assert Hq % Hkv == 0, (Hq, Hkv)
    return {
        "x": _w((lambda *s: _rng.normal(s) * 0.8)(B, Sq, D)),
        "k_cache": _w((lambda *s: _rng.normal(s) * 0.8)(B, Hkv, Sk, Dh)),
        "v_cache": _w((lambda *s: _rng.normal(s) * 0.05)(B, Hkv, Sk, Dh)),
        "wq": _w((lambda *s: _rng.normal(s) * 0.8)(D, Hq * Dh) * (D ** -0.5)),
        "wo": _w((lambda *s: _rng.normal(s) * 0.05)(Hq * Dh, D) * ((Hq * Dh) ** -0.5)),
    }

def reference(x, k_cache, v_cache, wq, wo):
    B, Sq, D = x.shape
    Hq, Dh = 16, 256
    Hkv = k_cache.shape[1]
    rep = Hq // Hkv
    q = (lambda x, *d: x.transpose(*d))((x @ wq).reshape(B, Sq, Hq, Dh), 0, 2, 1, 3)
    k = jnp.repeat(k_cache, rep, axis=1)
    v = jnp.repeat(v_cache, rep, axis=1)
    scores = jnp.einsum("bhqd,bhkd->bhqk", q, k) * (Dh ** -0.5)
    p = _softmax(scores, axis=-1)
    o = jnp.einsum("bhqk,bhkd->bhqd", p, v)
    return (lambda x, *d: x.transpose(*d))(o, 0, 2, 1, 3).reshape(B, Sq, Hq * Dh) @ wo
```

```python
import functools

import jax
import jax.numpy as jnp
import jax.experimental.pallas as pl
import jax.experimental.pallas.tpu as pltpu


def _kernel(x_ref, k_ref, v_ref, wq_ref, wo_ref, o_ref, q_scr, o_scr, *, Sq, Hkv, rep, Dh):
    scale = Dh ** -0.5
    x = x_ref[0]
    q = jnp.dot(x, wq_ref[...], preferred_element_type=jnp.float32)
    q_scr[...] = (q * scale).astype(jnp.bfloat16)
    for g in range(Hkv):
        qg = jnp.concatenate(
            [q_scr[:, (g * rep + r) * Dh:(g * rep + r + 1) * Dh] for r in range(rep)], axis=0)
        s = jax.lax.dot_general(qg, k_ref[0, g], (((1,), (1,)), ((), ())),
                                preferred_element_type=jnp.float32)
        m = jnp.max(s, axis=-1, keepdims=True)
        p = jnp.exp(s - m)
        l = jnp.sum(p, axis=-1, keepdims=True)
        o = jnp.dot(p.astype(jnp.bfloat16), v_ref[0, g], preferred_element_type=jnp.float32)
        o = (o * (1.0 / l)).astype(jnp.bfloat16)
        for r in range(rep):
            o_scr[:, (g * rep + r) * Dh:(g * rep + r + 1) * Dh] = o[r * Sq:(r + 1) * Sq]
    o_ref[0] = jnp.dot(o_scr[...], wo_ref[...], preferred_element_type=jnp.float32).astype(o_ref.dtype)


@jax.jit
def pallas_standalone__gqa_block_cached__near_ridge_kernel(x, k_cache, v_cache, wq, wo):
    B, Sq, D = x.shape
    _, Hkv, Sk, Dh = k_cache.shape
    Hq = wq.shape[1] // Dh
    rep = Hq // Hkv
    kern = functools.partial(_kernel, Sq=Sq, Hkv=Hkv, rep=rep, Dh=Dh)
    return pl.pallas_call(
        kern,
        grid=(B,),
        in_specs=[
            pl.BlockSpec((1, Sq, D), lambda b: (b, 0, 0)),
            pl.BlockSpec((1, Hkv, Sk, Dh), lambda b: (b, 0, 0, 0)),
            pl.BlockSpec((1, Hkv, Sk, Dh), lambda b: (b, 0, 0, 0)),
            pl.BlockSpec((D, Hq * Dh), lambda b: (0, 0)),
            pl.BlockSpec((Hq * Dh, D), lambda b: (0, 0)),
        ],
        out_specs=pl.BlockSpec((1, Sq, D), lambda b: (b, 0, 0)),
        out_shape=jax.ShapeDtypeStruct((B, Sq, D), x.dtype),
        scratch_shapes=[
            pltpu.VMEM((Sq, Hq * Dh), jnp.bfloat16),
            pltpu.VMEM((Sq, Hq * Dh), jnp.bfloat16),
        ],
        compiler_params=pltpu.CompilerParams(
            dimension_semantics=("arbitrary",),
            vmem_limit_bytes=100 * 1024 * 1024,
        ),
    )(x, k_cache, v_cache, wq, wo)
```

```python
import functools

import jax
import jax.numpy as jnp
from jax import lax
import jax.experimental.pallas as pl
import jax.experimental.pallas.tpu as pltpu

LOG2E = 1.4426950408889634
TT = 128
NS = 3
LEAD = 2
LAG = 1


def _kernel(x_hbm, k_hbm, v_hbm, wq_hbm, wot_hbm, out_hbm,
            x_v, wq_v, wot_v, k_v, v_v, q_carry, o_all, out_v,
            sem_wq, sem_wo, sem_x, sem_kv, sem_out, *, B, Sq, Hkv, rep, Dh):
    n_tiles = (B * Sq) // TT
    qscale = (Dh ** -0.5) * LOG2E
    gw = rep * Dh

    def x_copy(b):
        return pltpu.make_async_copy(x_hbm.at[b], x_v.at[b], sem_x.at[b])

    def kv_copies(b):
        slot = b % NS
        return (pltpu.make_async_copy(k_hbm.at[b], k_v.at[slot], sem_kv.at[0, slot]),
                pltpu.make_async_copy(v_hbm.at[b], v_v.at[slot], sem_kv.at[1, slot]))

    def wq_copy(i):
        cols = pl.ds(0, LEAD * gw) if i == 0 else pl.ds(LEAD * gw, (Hkv - LEAD) * gw)
        return pltpu.make_async_copy(wq_hbm.at[:, cols], wq_v.at[:, cols], sem_wq.at[i])

    def out_copy(t):
        rows = pl.ds(pl.multiple_of(t * TT, TT), TT)
        return pltpu.make_async_copy(out_v.at[rows], out_hbm.at[rows], sem_out.at[0])

    co = pltpu.make_async_copy(wot_hbm, wot_v, sem_wo.at[0])

    def qp(x, g):
        q = jnp.dot(x, wq_v[:, g * gw:(g + 1) * gw], preferred_element_type=jnp.float32)
        q = (q * qscale).astype(jnp.bfloat16)
        return jnp.concatenate([q[:, r * Dh:(r + 1) * Dh] for r in range(rep)], axis=0)

    def otile(t):
        rows = pl.ds(pl.multiple_of(t * TT, TT), TT)
        r = lax.dot_general(wot_v[...], o_all[rows, :], (((1,), (1,)), ((), ())),
                            preferred_element_type=jnp.float32)
        out_v[rows, :] = r.T.astype(out_v.dtype)
        out_copy(t).start()

    x_copy(0).start()
    wq_copy(0).start()
    x_copy(1).start()
    x_copy(2).start()
    wq_copy(1).start()
    for c in kv_copies(0):
        c.start()
    x_copy(0).wait()
    wq_copy(0).wait()
    x0 = x_v[0]
    for g in range(LEAD):
        q_carry[g] = qp(x0, g)
    wq_copy(1).wait()
    for c in kv_copies(1):
        c.start()

    def attn(b, t):
        slot = b % NS

        @pl.when(b + 3 < B)
        def _():
            x_copy(b + 3).start()

        @pl.when(b + 2 < B)
        def _():
            for c in kv_copies(b + 2):
                c.start()

        @pl.when(b == 1)
        def _():
            co.start()

        if t is not None:
            otile(t)

        x = x_v[b]
        x_nxt = x_v[jnp.minimum(b + 1, B - 1)]
        row0 = pl.multiple_of(b * Sq, 16)

        def qk(q, g):
            return lax.dot_general(q, k_v[slot, g], (((1,), (1,)), ((), ())),
                                   preferred_element_type=jnp.float32)

        def soft(s):
            m = jnp.max(s, axis=-1, keepdims=True)
            p = jnp.exp2(s - m)
            l = jnp.sum(p, axis=-1, keepdims=True)
            return (p * pl.reciprocal(l, approx=False)).astype(jnp.bfloat16)

        def pv(p, g):
            o = jnp.dot(p, v_v[slot, g], preferred_element_type=jnp.float32).astype(jnp.bfloat16)
            for r in range(rep):
                c0 = (g * rep + r) * Dh
                o_all[pl.ds(row0, Sq), c0:c0 + Dh] = o[r * Sq:(r + 1) * Sq]

        q = [None] * Hkv
        s = [None] * Hkv
        for g in range(LEAD):
            q[g] = q_carry[g]
        s[0] = qk(q[0], 0)
        for g in range(Hkv):
            if g + LEAD < Hkv:
                q[g + LEAD] = qp(x, g + LEAD)
            if g + 1 < Hkv:
                s[g + 1] = qk(q[g + 1], g + 1)
            p = soft(s[g])
            if g + LEAD >= Hkv:
                q_carry[g + LEAD - Hkv] = qp(x_nxt, g + LEAD - Hkv)
            pv(p, g)

    def body(b, carry):
        for c in kv_copies(b):
            c.wait()

        @pl.when(b + 1 < B)
        def _():
            x_copy(b + 1).wait()

        bp = b - LAG
        avail = (bp * Sq) // TT
        has_tile = jnp.logical_and(bp >= 1, avail > ((bp - 1) * Sq) // TT)

        @pl.when(jnp.logical_and(has_tile, avail == 1))
        def _():
            co.wait()

        @pl.when(has_tile)
        def _():
            attn(b, avail - 1)

        @pl.when(jnp.logical_not(has_tile))
        def _():
            attn(b, None)

        return carry

    lax.fori_loop(0, B, body, 0)
    done = ((B - 1 - LAG) * Sq) // TT
    for t in range(done, n_tiles):
        otile(t)
    for t in range(n_tiles):
        out_copy(t).wait()


@jax.jit
def pallas_standalone__gqa_block_cached__near_ridge_kernel(x, k_cache, v_cache, wq, wo):
    B, Sq, D = x.shape
    _, Hkv, Sk, Dh = k_cache.shape
    Hq = wq.shape[1] // Dh
    rep = Hq // Hkv
    kern = functools.partial(_kernel, B=B, Sq=Sq, Hkv=Hkv, rep=rep, Dh=Dh)
    bf = jnp.bfloat16
    any_spec = pl.BlockSpec(memory_space=pl.ANY)
    out = pl.pallas_call(
        kern,
        in_specs=[any_spec] * 5,
        out_specs=any_spec,
        out_shape=jax.ShapeDtypeStruct((B * Sq, D), x.dtype),
        scratch_shapes=[
            pltpu.VMEM((B, Sq, D), bf),
            pltpu.VMEM((D, Hq * Dh), bf),
            pltpu.VMEM((D, Hq * Dh), bf),
            pltpu.VMEM((NS, Hkv, Sk, Dh), bf),
            pltpu.VMEM((NS, Hkv, Sk, Dh), bf),
            pltpu.VMEM((LEAD, rep * Sq, Dh), bf),
            pltpu.VMEM((B * Sq, Hq * Dh), bf),
            pltpu.VMEM((B * Sq, D), bf),
            pltpu.SemaphoreType.DMA((2,)),
            pltpu.SemaphoreType.DMA((1,)),
            pltpu.SemaphoreType.DMA((B,)),
            pltpu.SemaphoreType.DMA((2, NS)),
            pltpu.SemaphoreType.DMA((1,)),
        ],
        compiler_params=pltpu.CompilerParams(vmem_limit_bytes=110 * 1024 * 1024,
                                             disable_bounds_checks=True),
        name="gqa_kernel",
    )(x, k_cache, v_cache, wq, wo.T)
    return out.reshape(B, Sq, D)
```

```python
import functools

import jax
import jax.numpy as jnp
from jax import lax
import jax.experimental.pallas as pl
import jax.experimental.pallas.tpu as pltpu

LOG2E = 1.4426950408889634
TT = 128
NS = 4
LEAD = 2
NPRE = 5
NB = 7
XPRE = NPRE
XD = 3
NXS = 8
WQ_FETCH = ((2, 3), (3, 5), (5, 8), (0, 2))
WO_AT = NPRE + 3
EPI_UNROLL = 2


def _kernel(x_hbm, k_hbm, v_hbm, wq_hbm, wot_hbm, out_hbm,
            x_v, wq_v, wot_v, k_v, v_v, q_carry, q_pre, o_all, out_v,
            sems, *, B, Sq, Hkv, rep, Dh):
    n_tiles = (B * Sq) // TT
    qscale = (Dh ** -0.5) * LOG2E
    gw = rep * Dh
    S_WQ = 0
    S_WO = S_WQ + len(WQ_FETCH)
    S_X0 = S_WO + 1
    S_OUT = S_X0 + 1
    S_X = S_OUT + 1
    S_K = S_X + NXS
    S_V = S_K + NS

    x_first = pltpu.make_async_copy(x_hbm.at[pl.ds(0, XPRE)], x_v.at[pl.ds(0, XPRE)], sems.at[S_X0])

    def x_copy(b):
        return pltpu.make_async_copy(x_hbm.at[b], x_v.at[b], sems.at[S_X + (b & (NXS - 1))])

    def kv_copies(b):
        slot = b & (NS - 1)
        return (pltpu.make_async_copy(k_hbm.at[b], k_v.at[slot], sems.at[S_K + slot]),
                pltpu.make_async_copy(v_hbm.at[b], v_v.at[slot], sems.at[S_V + slot]))

    def wq_copy(i):
        lo, hi = WQ_FETCH[i]
        cols = pl.ds(lo * gw, (hi - lo) * gw)
        return pltpu.make_async_copy(wq_hbm.at[:, cols], wq_v.at[:, cols], sems.at[S_WQ + i])

    def out_copy(t):
        rows = pl.ds(pl.multiple_of(t * TT, TT), TT)
        return pltpu.make_async_copy(out_v.at[rows], out_hbm.at[rows], sems.at[S_OUT])

    co = pltpu.make_async_copy(wot_hbm, wot_v, sems.at[S_WO])

    def qproj(x, g):
        q = jnp.dot(x, wq_v[:, g * gw:(g + 1) * gw], preferred_element_type=jnp.float32)
        return (q * qscale).astype(jnp.bfloat16)

    def stack_heads(q):
        return jnp.concatenate([q[:, r * Dh:(r + 1) * Dh] for r in range(rep)], axis=0)

    def qp(x, g):
        return stack_heads(qproj(x, g))

    def otile(t):
        rows = pl.ds(pl.multiple_of(t * TT, TT), TT)
        r = lax.dot_general(wot_v[...], o_all[rows, :], (((1,), (1,)), ((), ())),
                            preferred_element_type=jnp.float32)
        out_v[rows, :] = r.T.astype(out_v.dtype)
        out_copy(t).start()

    def when_in(idx, lo, hi, fn):
        pl.when(jnp.logical_and(idx >= lo, idx < hi))(fn)

    def start_fetch(b):
        when_in(b + XD, XPRE, B, lambda: x_copy(b + XD).start())

        def kv():
            for c in kv_copies(b + 2):
                c.start()
        when_in(b + 2, 0, B, kv)

    def wait_inputs(b):
        for c in kv_copies(b):
            c.wait()
        when_in(b + 1, XPRE, B, lambda: x_copy(b + 1).wait())

    def attn(b, q_lead, pre):
        slot = b & (NS - 1)
        x = x_v[b]
        x_nxt = x_v[jnp.minimum(b + 1, B - 1)]
        row0 = pl.multiple_of(b * Sq, 16)

        def qk(q, g):
            return lax.dot_general(q, k_v[slot, g], (((1,), (1,)), ((), ())),
                                   preferred_element_type=jnp.float32)

        def soft(s):
            m = jnp.max(s, axis=-1, keepdims=True)
            p = jnp.exp2(s - m)
            l = jnp.sum(p, axis=-1, keepdims=True)
            return (p * pl.reciprocal(l, approx=False)).astype(jnp.bfloat16)

        def pv(p, g):
            o = jnp.dot(p, v_v[slot, g], preferred_element_type=jnp.float32).astype(jnp.bfloat16)
            for r in range(rep):
                c0 = (g * rep + r) * Dh
                o_all[pl.ds(row0, Sq), c0:c0 + Dh] = o[r * Sq:(r + 1) * Sq]

        q = list(q_lead) + [None] * (Hkv - LEAD)
        s = [None] * Hkv
        nxt = []
        s[0] = qk(q[0], 0)
        for g in range(Hkv):
            if g + LEAD < Hkv:
                q[g + LEAD] = q_pre[b, g] if pre else qp(x, g + LEAD)
            if g + 1 < Hkv:
                s[g + 1] = qk(q[g + 1], g + 1)
            p = soft(s[g])
            if g + LEAD >= Hkv:
                nxt.append(qp(x_nxt, g + LEAD - Hkv))
            pv(p, g)
        return nxt

    def run(b0, nbatch, tiles, pre, start_wo=False):
        for i in range(nbatch):
            wait_inputs(b0 + i)
        for i in range(nbatch):
            start_fetch(b0 + i)
        if start_wo:
            pl.when(b0 == WO_AT)(co.start)
        for t in tiles:
            otile(t)
        ql = [q_carry[g] for g in range(LEAD)]
        for i in range(nbatch):
            ql = attn(b0 + i, ql, pre)
        for g in range(LEAD):
            q_carry[g] = ql[g]

    x_first.start()
    for i in range(len(WQ_FETCH)):
        wq_copy(i).start()
    for b in range(2):
        for c in kv_copies(b):
            c.start()
    x_first.wait()
    for i in range(len(WQ_FETCH)):
        wq_copy(i).wait()
        lo, hi = WQ_FETCH[i]
        for g in range(lo, hi):
            if g < LEAD:
                q_carry[g] = qp(x_v[0], g)
            else:
                xs = x_v[0:NPRE].reshape(NPRE * Sq, x_v.shape[-1])
                q = qproj(xs, g)
                for b in range(NPRE):
                    q_pre[b, g - LEAD] = stack_heads(q[b * Sq:(b + 1) * Sq])

    def c_body(b, carry):
        run(b, 1, (), True)
        return carry

    def b_body(b, carry):
        run(b, 1, (), False, start_wo=True)
        return carry

    first_a = NPRE + NB

    def a_body(i, carry):
        b = first_a + 2 * i
        run(b, 2, (2 * i, 2 * i + 1), False)
        return carry

    n_a = (B - first_a) // 2
    assert first_a + 2 * n_a == B
    lax.fori_loop(0, NPRE, c_body, 0)
    lax.fori_loop(NPRE, first_a, b_body, 0)
    co.wait()
    lax.fori_loop(0, n_a, a_body, 0)
    done = 2 * n_a

    def epi(i, carry):
        for j in range(EPI_UNROLL):
            otile(done + EPI_UNROLL * i + j)
        return carry

    assert (n_tiles - done) % EPI_UNROLL == 0
    lax.fori_loop(0, (n_tiles - done) // EPI_UNROLL, epi, 0)
    for t in range(n_tiles):
        out_copy(t).wait()


@jax.jit
def pallas_standalone__gqa_block_cached__near_ridge_kernel(x, k_cache, v_cache, wq, wo):
    B, Sq, D = x.shape
    _, Hkv, Sk, Dh = k_cache.shape
    Hq = wq.shape[1] // Dh
    rep = Hq // Hkv
    kern = functools.partial(_kernel, B=B, Sq=Sq, Hkv=Hkv, rep=rep, Dh=Dh)
    bf = jnp.bfloat16
    any_spec = pl.BlockSpec(memory_space=pl.ANY)
    n_sems = len(WQ_FETCH) + 3 + NXS + 2 * NS
    out = pl.pallas_call(
        kern,
        in_specs=[any_spec] * 5,
        out_specs=any_spec,
        out_shape=jax.ShapeDtypeStruct((B * Sq, D), x.dtype),
        scratch_shapes=[
            pltpu.VMEM((B, Sq, D), bf),
            pltpu.VMEM((D, Hq * Dh), bf),
            pltpu.VMEM((D, Hq * Dh), bf),
            pltpu.VMEM((NS, Hkv, Sk, Dh), bf),
            pltpu.VMEM((NS, Hkv, Sk, Dh), bf),
            pltpu.VMEM((LEAD, rep * Sq, Dh), bf),
            pltpu.VMEM((NPRE, Hkv - LEAD, rep * Sq, Dh), bf),
            pltpu.VMEM((B * Sq, Hq * Dh), bf),
            pltpu.VMEM((B * Sq, D), bf),
            pltpu.SemaphoreType.DMA((n_sems,)),
        ],
        compiler_params=pltpu.CompilerParams(vmem_limit_bytes=110 * 1024 * 1024,
                                             disable_bounds_checks=True),
        name="gqa_kernel",
    )(x, k_cache, v_cache, wq, wo.T)
    return out.reshape(B, Sq, D)
```

```python
import functools

import jax
import jax.numpy as jnp
from jax import lax
import jax.experimental.pallas as pl
import jax.experimental.pallas.tpu as pltpu

LOG2E = 1.4426950408889634
TT = 128
NS = 4
LEAD = 1
NPRE = 6
NB = 6
XA = 2
XD = 3
NXS = 8
QCH = 2
WO_AT = NPRE + 1
EPI_UNROLL = 4


def _kernel(x_hbm, k_hbm, v_hbm, wq_hbm, wot_hbm, out_hbm,
            x_v, wq_v, wot_v, k_v, v_v, q_carry, q_pre, o_all, out_v,
            sems, *, B, Sq, Hkv, rep, Dh):
    n_tiles = (B * Sq) // TT
    qscale = (Dh ** -0.5) * LOG2E
    gw = rep * Dh
    S_WQ = 0
    S_WO = S_WQ + Hkv
    S_X0 = S_WO + 1
    S_OUT = S_X0 + 2
    S_X = S_OUT + 1
    S_K = S_X + NXS
    S_V = S_K + NS

    def x_first(i):
        lo, hi = ((0, XA), (XA, NPRE))[i]
        rows = pl.ds(lo, hi - lo)
        return pltpu.make_async_copy(x_hbm.at[rows], x_v.at[rows], sems.at[S_X0 + i])

    def x_copy(b):
        return pltpu.make_async_copy(x_hbm.at[b], x_v.at[b], sems.at[S_X + (b & (NXS - 1))])

    def kv_copies(b):
        slot = b & (NS - 1)
        return (pltpu.make_async_copy(k_hbm.at[b], k_v.at[slot], sems.at[S_K + slot]),
                pltpu.make_async_copy(v_hbm.at[b], v_v.at[slot], sems.at[S_V + slot]))

    def wq_issue(g):
        return pltpu.make_async_copy(wq_hbm.at[:, pl.ds(g * gw, gw)], wq_v.at[g], sems.at[S_WQ + g])

    def wq_wait(g):
        pltpu.make_async_copy(wq_v.at[g], wq_v.at[g], sems.at[S_WQ + g]).wait()

    def out_copy(t):
        rows = pl.ds(pl.multiple_of(t * TT, TT), TT)
        return pltpu.make_async_copy(out_v.at[rows], out_hbm.at[rows], sems.at[S_OUT])

    co = pltpu.make_async_copy(wot_hbm, wot_v, sems.at[S_WO])

    def qproj(x, g):
        q = jnp.dot(x, wq_v[g], preferred_element_type=jnp.float32)
        return (q * qscale).astype(jnp.bfloat16)

    def stack_heads(q):
        return jnp.concatenate([q[:, r * Dh:(r + 1) * Dh] for r in range(rep)], axis=0)

    def qp(x, g):
        return stack_heads(qproj(x, g))

    def otile(t):
        rows = pl.ds(pl.multiple_of(t * TT, TT), TT)
        r = lax.dot_general(wot_v[...], o_all[rows, :], (((1,), (1,)), ((), ())),
                            preferred_element_type=jnp.float32)
        out_v[rows, :] = r.T.astype(out_v.dtype)
        out_copy(t).start()

    def when_in(idx, lo, hi, fn):
        pl.when(jnp.logical_and(idx >= lo, idx < hi))(fn)

    def start_fetch(b):
        when_in(b + XD, NPRE, B, lambda: x_copy(b + XD).start())

        def kv():
            for c in kv_copies(b + 2):
                c.start()
        when_in(b + 2, 0, B, kv)

    def wait_inputs(b):
        for c in kv_copies(b):
            c.wait()
        when_in(b + 1, NPRE, B, lambda: x_copy(b + 1).wait())

    def attn(b, q_lead, pre):
        slot = b & (NS - 1)
        x = x_v[b]
        x_nxt = x_v[jnp.minimum(b + 1, B - 1)]
        row0 = pl.multiple_of(b * Sq, 16)

        def qk(q, g):
            return lax.dot_general(q, k_v[slot, g], (((1,), (1,)), ((), ())),
                                   preferred_element_type=jnp.float32)

        def soft(s):
            m = jnp.max(s, axis=-1, keepdims=True)
            p = jnp.exp2(s - m)
            l = jnp.sum(p, axis=-1, keepdims=True)
            return (p * pl.reciprocal(l, approx=False)).astype(jnp.bfloat16)

        def pv(p, g):
            o = jnp.dot(p, v_v[slot, g], preferred_element_type=jnp.float32).astype(jnp.bfloat16)
            for r in range(rep):
                c0 = (g * rep + r) * Dh
                o_all[pl.ds(row0, Sq), c0:c0 + Dh] = o[r * Sq:(r + 1) * Sq]

        q = list(q_lead) + [None] * (Hkv - LEAD)
        s = [None] * Hkv
        nxt = []
        s[0] = qk(q[0], 0)
        for g in range(Hkv):
            if g + LEAD < Hkv:
                q[g + LEAD] = q_pre[b, g] if pre else qp(x, g + LEAD)
            if g + 1 < Hkv:
                s[g + 1] = qk(q[g + 1], g + 1)
            p = soft(s[g])
            if g + LEAD >= Hkv:
                nxt.append(qp(x_nxt, g + LEAD - Hkv))
            pv(p, g)
        return nxt

    def run(b0, nbatch, tiles, pre, start_wo=False):
        for i in range(nbatch):
            wait_inputs(b0 + i)
        for i in range(nbatch):
            start_fetch(b0 + i)
        if start_wo:
            pl.when(b0 == WO_AT)(co.start)
        for t in tiles:
            otile(t)
        ql = [q_carry[g] for g in range(LEAD)]
        for i in range(nbatch):
            ql = attn(b0 + i, ql, pre)
        for g in range(LEAD):
            q_carry[g] = ql[g]

    def pre_q(g, lo, hi):
        xs = x_v[lo:hi].reshape((hi - lo) * Sq, x_v.shape[-1])
        q = qproj(xs, g)
        for b in range(lo, hi):
            q_pre[b, g - LEAD] = stack_heads(q[(b - lo) * Sq:(b - lo + 1) * Sq])

    x_first(0).start()
    wq_issue(LEAD).start()
    x_first(1).start()
    for g in list(range(LEAD + 1, Hkv)) + list(range(LEAD)):
        wq_issue(g).start()
    for b in range(2):
        for c in kv_copies(b):
            c.start()
    x_first(0).wait()
    wq_wait(LEAD)
    pre_q(LEAD, 0, XA)
    x_first(1).wait()
    pre_q(LEAD, XA, NPRE)

    def q_body(i, carry):
        g0 = LEAD + 1 + QCH * i
        for j in range(QCH):
            wq_wait(g0 + j)
        for j in range(QCH):
            pre_q(g0 + j, 0, NPRE)
        return carry

    assert (Hkv - LEAD - 1) % QCH == 0
    lax.fori_loop(0, (Hkv - LEAD - 1) // QCH, q_body, 0)
    for g in range(LEAD):
        wq_wait(g)
    for g in range(LEAD):
        q_carry[g] = qp(x_v[0], g)

    def c_body(b, carry):
        run(b, 1, (), True)
        return carry

    def b_body(b, carry):
        run(b, 1, (), False, start_wo=True)
        return carry

    first_a = NPRE + NB

    def a_body(i, carry):
        b = first_a + 2 * i
        run(b, 2, (2 * i, 2 * i + 1), False)
        return carry

    n_a = (B - first_a) // 2
    assert first_a + 2 * n_a == B
    lax.fori_loop(0, NPRE, c_body, 0)
    lax.fori_loop(NPRE, first_a, b_body, 0)
    co.wait()
    lax.fori_loop(0, n_a, a_body, 0)
    done = 2 * n_a

    def epi(i, carry):
        for j in range(EPI_UNROLL):
            otile(done + EPI_UNROLL * i + j)
        return carry

    assert (n_tiles - done) % EPI_UNROLL == 0
    lax.fori_loop(0, (n_tiles - done) // EPI_UNROLL, epi, 0)
    for t in range(n_tiles):
        out_copy(t).wait()


@jax.jit
def pallas_standalone__gqa_block_cached__near_ridge_kernel(x, k_cache, v_cache, wq, wo):
    B, Sq, D = x.shape
    _, Hkv, Sk, Dh = k_cache.shape
    Hq = wq.shape[1] // Dh
    rep = Hq // Hkv
    kern = functools.partial(_kernel, B=B, Sq=Sq, Hkv=Hkv, rep=rep, Dh=Dh)
    bf = jnp.bfloat16
    any_spec = pl.BlockSpec(memory_space=pl.ANY)
    n_sems = Hkv + 4 + NXS + 2 * NS
    out = pl.pallas_call(
        kern,
        in_specs=[any_spec] * 5,
        out_specs=any_spec,
        out_shape=jax.ShapeDtypeStruct((B * Sq, D), x.dtype),
        scratch_shapes=[
            pltpu.VMEM((B, Sq, D), bf),
            pltpu.VMEM((Hkv, D, rep * Dh), bf),
            pltpu.VMEM((D, Hq * Dh), bf),
            pltpu.VMEM((NS, Hkv, Sk, Dh), bf),
            pltpu.VMEM((NS, Hkv, Sk, Dh), bf),
            pltpu.VMEM((LEAD, rep * Sq, Dh), bf),
            pltpu.VMEM((NPRE, Hkv - LEAD, rep * Sq, Dh), bf),
            pltpu.VMEM((B * Sq, Hq * Dh), bf),
            pltpu.VMEM((B * Sq, D), bf),
            pltpu.SemaphoreType.DMA((n_sems,)),
        ],
        compiler_params=pltpu.CompilerParams(vmem_limit_bytes=110 * 1024 * 1024,
                                             disable_bounds_checks=True),
        name="gqa_kernel",
    )(x, k_cache, v_cache, wq, wo.T)
    return out.reshape(B, Sq, D)
```

```python
import functools

import jax
import jax.numpy as jnp
from jax import lax
import jax.experimental.pallas as pl
import jax.experimental.pallas.tpu as pltpu

LOG2E = 1.4426950408889634
TT = 128
NS = 4
LEAD = 1
NPRE = 6
NB = 6
XA = 2
XD = 3
NXS = 8
QCH = 2
WO_AT = NPRE + 1
EPI_UNROLL = 4


def _kernel(x_hbm, k_hbm, v_hbm, wq_hbm, wot_hbm, out_hbm,
            x_v, wq_v, wot_v, k_v, v_v, q_carry, q_pre, o_all, out_v,
            sems, *, B, Sq, Hkv, rep, Dh):
    n_tiles = (B * Sq) // TT
    qscale = (Dh ** -0.5) * LOG2E
    gw = rep * Dh
    S_WQ = 0
    S_WO = S_WQ + Hkv
    S_X0 = S_WO + 1
    S_OUT = S_X0 + 2
    S_X = S_OUT + 1
    S_K = S_X + NXS
    S_V = S_K + NS

    def x_first(i):
        lo, hi = ((0, XA), (XA, NPRE))[i]
        rows = pl.ds(lo, hi - lo)
        return pltpu.make_async_copy(x_hbm.at[rows], x_v.at[rows], sems.at[S_X0 + i])

    def x_copy(b):
        return pltpu.make_async_copy(x_hbm.at[b], x_v.at[b], sems.at[S_X + (b & (NXS - 1))])

    def kv_copies(b):
        slot = b & (NS - 1)
        return (pltpu.make_async_copy(k_hbm.at[b], k_v.at[slot], sems.at[S_K + slot]),
                pltpu.make_async_copy(v_hbm.at[b], v_v.at[slot], sems.at[S_V + slot]))

    def wq_start(g):
        pltpu.make_async_copy(wq_hbm.at[:, pl.ds(g * gw, gw)], wq_v.at[g], sems.at[S_WQ + g]).start()

    def wq_wait(g):
        pltpu.make_async_copy(wq_v.at[g], wq_v.at[g], sems.at[S_WQ + g]).wait()

    def out_copy(t):
        rows = pl.ds(pl.multiple_of(t * TT, TT), TT)
        return pltpu.make_async_copy(out_v.at[rows], out_hbm.at[rows], sems.at[S_OUT])

    wo_copy = pltpu.make_async_copy(wot_hbm, wot_v, sems.at[S_WO])

    def qproj(x, g):
        q = jnp.dot(x, wq_v[g], preferred_element_type=jnp.float32)
        return (q * qscale).astype(jnp.bfloat16)

    def stack_heads(q):
        return jnp.concatenate([q[:, r * Dh:(r + 1) * Dh] for r in range(rep)], axis=0)

    def qp(x, g):
        return stack_heads(qproj(x, g))

    def otile(t):
        rows = pl.ds(pl.multiple_of(t * TT, TT), TT)
        r = lax.dot_general(wot_v[...], o_all[rows, :], (((1,), (1,)), ((), ())),
                            preferred_element_type=jnp.float32)
        out_v[rows, :] = r.T.astype(out_v.dtype)
        out_copy(t).start()

    def when_in(idx, lo, hi, fn):
        pl.when(jnp.logical_and(idx >= lo, idx < hi))(fn)

    def start_fetch(b):
        when_in(b + XD, NPRE, B, lambda: x_copy(b + XD).start())

        def kv():
            for c in kv_copies(b + 2):
                c.start()
        when_in(b + 2, 0, B, kv)

    def wait_inputs(b):
        for c in kv_copies(b):
            c.wait()
        when_in(b + 1, NPRE, B, lambda: x_copy(b + 1).wait())

    def attn(b, q_lead, pre):
        slot = b & (NS - 1)
        x = x_v[b]
        x_nxt = x_v[jnp.minimum(b + 1, B - 1)]
        row0 = pl.multiple_of(b * Sq, 16)

        def qk(q, g):
            return lax.dot_general(q, k_v[slot, g], (((1,), (1,)), ((), ())),
                                   preferred_element_type=jnp.float32)

        def soft(s):
            m = jnp.max(s, axis=-1, keepdims=True)
            p = jnp.exp2(s - m)
            l = jnp.sum(p, axis=-1, keepdims=True)
            return (p * pl.reciprocal(l, approx=False)).astype(jnp.bfloat16)

        def pv(p, g):
            o = jnp.dot(p, v_v[slot, g], preferred_element_type=jnp.float32).astype(jnp.bfloat16)
            for r in range(rep):
                c0 = (g * rep + r) * Dh
                o_all[pl.ds(row0, Sq), c0:c0 + Dh] = o[r * Sq:(r + 1) * Sq]

        q = list(q_lead) + [None] * (Hkv - LEAD)
        s = [None] * Hkv
        nxt = []
        s[0] = qk(q[0], 0)
        for g in range(Hkv):
            if g + LEAD < Hkv:
                q[g + LEAD] = q_pre[b, g] if pre else qp(x, g + LEAD)
            if g + 1 < Hkv:
                s[g + 1] = qk(q[g + 1], g + 1)
            p = soft(s[g])
            if g + LEAD >= Hkv:
                nxt.append(qp(x_nxt, g + LEAD - Hkv))
            pv(p, g)
        return nxt

    def run(b0, nbatch, tiles, pre, start_wo=False):
        for i in range(nbatch):
            wait_inputs(b0 + i)
        for i in range(nbatch):
            start_fetch(b0 + i)
        if start_wo:
            pl.when(b0 == WO_AT)(wo_copy.start)
        for t in tiles:
            otile(t)
        ql = [q_carry[g] for g in range(LEAD)]
        for i in range(nbatch):
            ql = attn(b0 + i, ql, pre)
        for g in range(LEAD):
            q_carry[g] = ql[g]

    def pre_q(g, lo, hi):
        xs = x_v[lo:hi].reshape((hi - lo) * Sq, x_v.shape[-1])
        q = qproj(xs, g)
        for b in range(lo, hi):
            q_pre[b, g - LEAD] = stack_heads(q[(b - lo) * Sq:(b - lo + 1) * Sq])

    x_first(0).start()
    wq_start(LEAD)
    x_first(1).start()
    for g in list(range(LEAD + 1, Hkv)) + list(range(LEAD)):
        wq_start(g)
    for b in range(2):
        for c in kv_copies(b):
            c.start()
    x_first(0).wait()
    wq_wait(LEAD)
    pre_q(LEAD, 0, XA)
    x_first(1).wait()
    pre_q(LEAD, XA, NPRE)

    def q_body(i, carry):
        g0 = LEAD + 1 + QCH * i
        for j in range(QCH):
            wq_wait(g0 + j)
        for j in range(QCH):
            pre_q(g0 + j, 0, NPRE)
        return carry

    assert (Hkv - LEAD - 1) % QCH == 0
    lax.fori_loop(0, (Hkv - LEAD - 1) // QCH, q_body, 0)
    for g in range(LEAD):
        wq_wait(g)
    for g in range(LEAD):
        q_carry[g] = qp(x_v[0], g)

    def c_body(b, carry):
        run(b, 1, (), True)
        return carry

    def b_body(b, carry):
        run(b, 1, (), False, start_wo=True)
        return carry

    first_a = NPRE + NB
    lax.fori_loop(0, NPRE, c_body, 0)
    lax.fori_loop(NPRE, first_a, b_body, 0)
    wo_copy.wait()

    def a_body(i, carry):
        run(first_a + 2 * i, 2, (2 * i, 2 * i + 1), False)
        return carry

    n_a = (B - first_a) // 2
    assert first_a + 2 * n_a == B
    assert all((2 * i + 2) * TT <= (first_a + 2 * i) * Sq for i in range(n_a))
    lax.fori_loop(0, n_a, a_body, 0)

    done = 2 * n_a

    def epi(i, carry):
        for j in range(EPI_UNROLL):
            otile(done + EPI_UNROLL * i + j)
        return carry

    assert (n_tiles - done) % EPI_UNROLL == 0
    lax.fori_loop(0, (n_tiles - done) // EPI_UNROLL, epi, 0)
    for t in range(n_tiles):
        out_copy(t).wait()


@jax.jit
def pallas_standalone__gqa_block_cached__near_ridge_kernel(x, k_cache, v_cache, wq, wo):
    B, Sq, D = x.shape
    _, Hkv, Sk, Dh = k_cache.shape
    Hq = wq.shape[1] // Dh
    rep = Hq // Hkv
    assert (B * Sq) % TT == 0 and Sq % 16 == 0
    kern = functools.partial(_kernel, B=B, Sq=Sq, Hkv=Hkv, rep=rep, Dh=Dh)
    bf = jnp.bfloat16
    any_spec = pl.BlockSpec(memory_space=pl.ANY)
    n_sems = Hkv + 4 + NXS + 2 * NS
    out = pl.pallas_call(
        kern,
        in_specs=[any_spec] * 5,
        out_specs=any_spec,
        out_shape=jax.ShapeDtypeStruct((B * Sq, D), x.dtype),
        scratch_shapes=[
            pltpu.VMEM((B, Sq, D), bf),
            pltpu.VMEM((Hkv, D, rep * Dh), bf),
            pltpu.VMEM((D, Hq * Dh), bf),
            pltpu.VMEM((NS, Hkv, Sk, Dh), bf),
            pltpu.VMEM((NS, Hkv, Sk, Dh), bf),
            pltpu.VMEM((LEAD, rep * Sq, Dh), bf),
            pltpu.VMEM((NPRE, Hkv - LEAD, rep * Sq, Dh), bf),
            pltpu.VMEM((B * Sq, Hq * Dh), bf),
            pltpu.VMEM((B * Sq, D), bf),
            pltpu.SemaphoreType.DMA((n_sems,)),
        ],
        compiler_params=pltpu.CompilerParams(vmem_limit_bytes=110 * 1024 * 1024,
                                             disable_bounds_checks=True,
                                             disable_semaphore_checks=True),
        name="gqa_kernel",
    )(x, k_cache, v_cache, wq, wo.T)
    return out.reshape(B, Sq, D)
```
